```python
import jax
import jax.numpy as jnp

def _softmax(x, axis=-1):
    return jax.nn.softmax(x, axis=axis)
def _gelu(x):
    return jax.nn.gelu(x, approximate=True)
def _silu(x):
    return jax.nn.silu(x)
def _sigmoid(x):
    return jax.nn.sigmoid(x)
def _layernorm(x, axis=-1, eps=1e-5):
    m = jnp.mean(x, axis=axis, keepdims=True)
    v = jnp.var(x, axis=axis, keepdims=True)
    return (x - m) / jnp.sqrt(v + eps)
def _scatter_add(tgt, idx, src, axis=0):
    return tgt.at[idx].add(src)
def _segment_sum(src, seg, n):
    return jax.ops.segment_sum(src, seg, n)
class _Rng:
    def __init__(self, key):
        self._k = key
    def _next(self):
        self._k, sub = jax.random.split(self._k)
        return sub
    def normal(self, shape):
        return jax.random.normal(self._next(), shape, dtype=jnp.bfloat16)
    def randint(self, lo, hi, shape):
        return jax.random.randint(self._next(), shape, lo, hi, dtype=jnp.int32)
    def uniform(self, shape, lo=0.0, hi=1.0):
        return jax.random.uniform(self._next(), shape, jnp.bfloat16, lo, hi)
    def permutation(self, n):
        return jax.random.permutation(self._next(), n)


kernel_name = 'recurrent_scan__sliding_block_cached__moe_arch_mod__decode'

def setup_inputs():
    _rng = _Rng(jax.random.key(int.from_bytes(__import__("os").urandom(4), "little")))
    _w = (lambda a: (lambda t: t.astype(jnp.bfloat16) if jnp.issubdtype(t.dtype, jnp.floating) else t)(jnp.asarray(a)))
    def _A_setup():
        B, Sq, D = 1, 1, 512
        Hq, Hkv, Sk, Dh = 32, 32, 32768, 128
        assert Hq % Hkv == 0, (Hq, Hkv)
        return {
            "x": _w((lambda *s: _rng.normal(s) * 0.05)(B, Sq, D)),
            "k_cache": _w((lambda *s: _rng.normal(s) * 0.05)(B, Hkv, Sk, Dh)),
            "v_cache": _w((lambda *s: _rng.normal(s) * 0.05)(B, Hkv, Sk, Dh)),
            "wq": _w((lambda *s: _rng.normal(s) * 0.05)(D, Hq * Dh) * (D ** -0.5)),
            "wo": _w((lambda *s: _rng.normal(s) * 0.05)(Hq * Dh, D) * ((Hq * Dh) ** -0.5)),
        }
    _A_in = _A_setup()

    def _B_setup():
        B, S, D, F, C = 1, 1, 512, 1376, 1
        return {
            "x": _w((lambda *s: _rng.normal(s) * 0.05)(B, S, D)),
            "w_r": _w((lambda *s: _rng.normal(s) * 0.05)(D)),
            "w_gate": _w((lambda *s: _rng.normal(s) * 0.05)(D, F)),
            "w_up": _w((lambda *s: _rng.normal(s) * 0.05)(D, F)),
            "w_down": _w((lambda *s: _rng.normal(s) * 0.05)(F, D)),
        }
    _B_in = _B_setup()

    return {
        "A_x": _A_in["x"],
        "A_k_cache": _A_in["k_cache"],
        "A_v_cache": _A_in["v_cache"],
        "A_wq": _A_in["wq"],
        "A_wo": _A_in["wo"],
        "B_x": _B_in["x"],
        "B_w_r": _B_in["w_r"],
        "B_w_gate": _B_in["w_gate"],
        "B_w_up": _B_in["w_up"],
        "B_w_down": _B_in["w_down"],
    }

def reference(A_x, A_k_cache, A_v_cache, A_wq, A_wo, B_x, B_w_r, B_w_gate, B_w_up, B_w_down):
    def _A_ref(x, k_cache, v_cache, wq, wo):
        B, Sq, D = x.shape
        Hq, Dh = 32, 128
        Hkv, Sk = k_cache.shape[1], k_cache.shape[2]
        W = min(4096, max(256, Sk // 4))
        rep = Hq // Hkv
        q = (lambda x, *d: x.transpose(*d))((x @ wq).reshape(B, Sq, Hq, Dh), 0, 2, 1, 3)
        k = jnp.repeat(k_cache[:, :, Sk - W:, :], rep, axis=1)
        v = jnp.repeat(v_cache[:, :, Sk - W:, :], rep, axis=1)
        scores = jnp.einsum("bhqd,bhkd->bhqk", q, k) * (Dh ** -0.5)
        p = _softmax(scores, axis=-1)
        o = jnp.einsum("bhqk,bhkd->bhqd", p, v)
        return (lambda x, *d: x.transpose(*d))(o, 0, 2, 1, 3).reshape(B, Sq, Hq * Dh) @ wo

    def _B_ref(x, w_r, w_gate, w_up, w_down):
        B, S, D = x.shape
        C = 1
        r = x @ w_r
        idx = jnp.argsort(-r, axis=-1)[:, :C]
        idx_e = jnp.repeat(idx.reshape(B, C, 1), D, axis=2)
        x_sel = jnp.take_along_axis(x, idx_e, axis=1)
        g = _silu(x_sel @ w_gate)
        u = x_sel @ w_up
        y = (g * u) @ w_down
        r_sel = _sigmoid(jnp.take_along_axis(r, idx, axis=1))
        y = y * r_sel.reshape(B, C, 1)
        b_off = (jnp.arange(B) * S).reshape(B, 1)
        flat_idx = (idx + b_off).reshape(B * C)
        zero = (x * 0.0).reshape(B * S, D)
        upd = _scatter_add(zero, flat_idx, y.reshape(B * C, D), axis=0)
        return x + upd.reshape(B, S, D)

    x = A_x
    xn = _layernorm(x, axis=-1)
    s = _A_ref(xn, A_k_cache, A_v_cache, A_wq, A_wo)
    g = _silu(_B_ref(xn, B_w_r, B_w_gate, B_w_up, B_w_down))
    return x + s * g
```

```python
import functools
import jax, jax.numpy as jnp
from jax import lax
from jax.experimental import pallas as pl
from jax.experimental.pallas import tpu as pltpu
import numpy as np

H, SK, DH, W, D, F = 32, 32768, 128, 4096, 512, 1376
LOG2E = 1.4426950408889634
NT = (((1,), (1,)), ((), ()))


def make(name="v6", GC=512, GD=128, DQ=40, D0=None, debug=False, nobc=False, nosc=True, vlimit=64, order="wwss", NH=32,
         ffn_down_at="p0", qparts=4, swap=False, scoped=False, unroll2=False):
    NKV = W // GD
    GB = GD * DH * 2
    WOR = GB // (D * 2)
    NWO = (DH // 2) // WOR
    NS = NKV + NWO
    GPR = GC // GD
    TPR = GC // 128
    D0 = DQ if D0 is None else D0
    assert DQ <= 2 * NS - GPR
    f32, bf16 = jnp.float32, jnp.bfloat16
    SC = (DH ** -0.5) * LOG2E
    PA, PB = (1, 0) if swap else (0, 1)
    scope = (lambda n: jax.named_scope(n)) if scoped else (lambda n: jax.named_scope("k"))

    def kernel(x_hbm, k_hbm, v_hbm, wq_hbm, wo_hbm, wr_hbm, wg_hbm, wu_hbm, wd_hbm, o_ref,
               xb, wrb, wqb, kb, vb, wob, wgb, wub, wdb, q_scr, semA, semB, semP, sem0):

        def par(h):
            return h % 2 if isinstance(h, int) else lax.rem(h, 2)

        def A_cp(h, j):
            p = par(h)
            if j < NKV:
                r = j * GD
                return pltpu.make_async_copy(k_hbm.at[0, h, pl.ds(SK - W + r, GD), :], kb.at[p, pl.ds(r, GD), :], semA.at[p, j])
            r = (j - NKV) * WOR
            r0 = (h - 1) * DH + r
            r0 = r0 if isinstance(h, int) else pl.multiple_of(r0, WOR)
            return pltpu.make_async_copy(wo_hbm.at[pl.ds(r0, WOR), :], wob.at[p, pl.ds(r, WOR), :], semA.at[p, j])

        def B_cp(h, j):
            p = par(h)
            if j < NKV:
                r = j * GD
                return pltpu.make_async_copy(v_hbm.at[0, h - 1, pl.ds(SK - W + r, GD), :], vb.at[p, pl.ds(r, GD), :], semB.at[p, j])
            r = DH // 2 + (j - NKV) * WOR
            r0 = (h - 1) * DH + r
            r0 = r0 if isinstance(h, int) else pl.multiple_of(r0, WOR)
            return pltpu.make_async_copy(wo_hbm.at[pl.ds(r0, WOR), :], wob.at[p, pl.ds(r, WOR), :], semB.at[p, j])

        CW = GB // (8 * 2)
        NCW = (H * DH) // CW
        nwq = (D // 8) * NCW
        FR = GB // (D * 2)
        nff_m = -(-F // FR)
        pa, pb = [], []
        for i in range(nwq):
            r8, c = i // NCW, i % NCW
            pa.append(("wq", i, pltpu.make_async_copy(wq_hbm.at[pl.ds(8 * r8, 8), pl.ds(c * CW, CW)],
                                                       wqb.at[pl.ds(8 * r8, 8), pl.ds(c * CW, CW)], semP.at[i])))
        for m, (src, dst) in enumerate(((wg_hbm, wgb), (wu_hbm, wub), (wd_hbm, wdb))):
            for i in range(nff_m):
                n = min(FR, F - i * FR)
                pb.append((("wg", "wu", "wd")[m], i, pltpu.make_async_copy(src.at[pl.ds(i * FR, n), :], dst.at[pl.ds(i * FR, n), :],
                                                                          semP.at[nwq + m * nff_m + i])))
        while len(pa) < len(pb):
            pa.append(None)
        for j in range(NKV):
            (pa if j % 2 == 0 else pb).append(("k0", j, A_cp(0, j)))
        NP = len(pa)
        assert len(pa) == len(pb)
        k0_done = set()

        def itemA(i):
            if i < NP:
                return None if pa[i] is None else pa[i][2]
            i -= NP
            h, j = 1 + i // NS, i % NS
            if h == 2 and j < NKV:
                assert j in k0_done, ("K(2) overwrites unconsumed K(0) group", j)
            assert h <= 2
            return A_cp(h, j)

        def itemB(i):
            if i < NP:
                return pb[i][2]
            i -= NP
            assert 1 + i // NS <= 2
            return B_cp(1 + i // NS, i % NS)

        issued = [0]

        def issue_upto(n):
            while issued[0] < n:
                c = itemA(issued[0])
                if c is not None:
                    c.start(priority=PA)
                itemB(issued[0]).start(priority=PB)
                issued[0] += 1

        c_x = pltpu.make_async_copy(x_hbm, xb, sem0.at[0])
        c_wr = pltpu.make_async_copy(wr_hbm, wrb, sem0.at[1])
        c_x.start()
        c_wr.start()
        issue_upto(D0)

        c_x.wait()
        x = xb[...].astype(f32).reshape(1, D)
        mean = jnp.mean(x, axis=-1, keepdims=True)
        xc = x - mean
        var = jnp.mean(xc * xc, axis=-1, keepdims=True)
        xn = xc / jnp.sqrt(var + 1e-5)
        xn_b1 = xn.astype(bf16)
        xn_b = jnp.broadcast_to(xn_b1, (8, D))
        c_wr.wait()
        r = jnp.sum(xn_b1.astype(f32) * wrb[...].astype(f32).reshape(1, D), axis=-1, keepdims=True)
        rs = jax.nn.sigmoid(r)

        rows = lax.broadcasted_iota(jnp.int32, (8, 128), 0)

        def k_compute(qb, p, reg, C):
            s = lax.dot_general(qb, kb[p, pl.ds(reg * GC, GC), :], NT, preferred_element_type=f32)
            for t in range(TPR):
                T = reg * TPR + t
                st = s[0:8, t * 128:(t + 1) * 128]
                i, rr = T // 8, T % 8
                C[i] = st if rr == 0 else jnp.where(rows == rr, st, C[i])

        def v_compute(P, p, reg, acc):
            for t in range(TPR):
                T = reg * TPR + t
                out = jnp.dot(P[(T // 16) * 16:(T // 16) * 16 + 16], vb[p, pl.ds(T * 128, 128), :], preferred_element_type=f32)
                hf = (T % 16) // 8
                sel = jnp.where(rows == T % 8, out[8 * hf:8 * hf + 8], 0.0)
                acc = sel if acc is None else acc + sel
            return acc

        def softmax_finish(C):
            Cm = jnp.concatenate(C, axis=0)
            m = jnp.max(Cm, axis=(0, 1), keepdims=True)
            p = jnp.exp2((Cm - m) * SC)
            l = jnp.sum(p, axis=(0, 1), keepdims=True)
            return p.astype(bf16), 1.0 / l

        def out_proj(o, linv, p):
            return jnp.dot((o * linv).astype(bf16), wob[p], preferred_element_type=f32)

        RQ = D // qparts
        st = dict(q=None, g=None, a=None, y=None, C=[None] * 4, qb=None)

        def ffn_down():
            y = jnp.dot(st["a"], wdb[...], preferred_element_type=f32)
            y = y * rs
            bb = xn + (xn * 0.0 + y)
            st["gg"] = bb * jax.nn.sigmoid(bb)

        for i in range(NP):
          with scope(f"P0_{i // 16:02d}"):
            la = D0 if i < NP - NKV // 2 else DQ
            for lst in (pa, pb):
                it = lst[i]
                if it is not None:
                    it[2].wait()
            issue_upto(max(issued[0], i + 1 + la))
            ita, itb = pa[i], pb[i]
            if ita is not None and ita[0] == "wq" and (ita[1] + 1) % (nwq // qparts) == 0:
                p = (ita[1] + 1) // (nwq // qparts) - 1
                t = jnp.dot(xn_b[:, p * RQ:(p + 1) * RQ], wqb[pl.ds(p * RQ, RQ), :], preferred_element_type=f32)
                st["q"] = t if st["q"] is None else st["q"] + t
                if p == qparts - 1:
                    for h in range(H):
                        q_scr[h] = st["q"][:, h * DH:(h + 1) * DH]
            if itb[0] == "wg" and itb[1] == nff_m - 1:
                st["g"] = lax.dot_general(xn_b, wgb[...], NT, preferred_element_type=f32)
            if itb[0] == "wu" and itb[1] == nff_m - 1:
                u = lax.dot_general(xn_b, wub[...], NT, preferred_element_type=f32)
                st["a"] = ((st["g"] * jax.nn.sigmoid(st["g"])) * u).astype(bf16)
            if itb[0] == "wd" and itb[1] == nff_m - 1 and ffn_down_at == "p0":
                ffn_down()
            if itb[0] == "k0" and (itb[1] + 1) % GPR == 0:
                if st["qb"] is None:
                    st["qb"] = q_scr[0].astype(bf16)
                k_compute(st["qb"], 0, itb[1] // GPR, st["C"])
                for j in range(itb[1] + 1 - GPR, itb[1] + 1):
                    k0_done.add(j)
        P, linv = softmax_finish(st["C"])
        if ffn_down_at == "p1":
            ffn_down()
        gg = st["gg"]
        assert issued[0] == NP + DQ, (issued, NP, DQ)

        def step(h, carry, static_tail=None):
            s_acc, P, linv = carry
            p = par(h)
            qb = q_scr[h].astype(bf16)
            C = [None] * 4
            o = None

            def issue(jj):
                k, j2 = jj // NS, jj % NS
                hh = h + k
                if isinstance(h, int):
                    if (j2 < NKV and hh < NH) or (j2 >= NKV and hh <= NH):
                        A_cp(hh, j2).start(priority=PA)
                    if hh <= NH:
                        B_cp(hh, j2).start(priority=PB)
                    return
                if j2 < NKV:
                    @pl.when(hh < NH)
                    def _():
                        A_cp(hh, j2).start(priority=PA)
                    if k == 0 or (k == 1):
                        B_cp(hh, j2).start(priority=PB)
                    else:
                        @pl.when(hh <= NH)
                        def _():
                            B_cp(hh, j2).start(priority=PB)
                else:
                    if k <= 1:
                        A_cp(hh, j2).start(priority=PA)
                        B_cp(hh, j2).start(priority=PB)
                    else:
                        @pl.when(hh <= NH)
                        def _():
                            A_cp(hh, j2).start(priority=PA)
                            B_cp(hh, j2).start(priority=PB)

            def ia(jj):
                pass
            for j in range(NS):
              with scope(f"S_{j // 8}"):
                A_cp(h, j).wait()
                B_cp(h, j).wait()
                issue(j + DQ)
                if j < NKV and (j + 1) % GPR == 0:
                    k_compute(qb, p, j // GPR, C)
                    o = v_compute(P, p, j // GPR, o)
            s_acc = s_acc + out_proj(o, linv, p)
            P, linv = softmax_finish(C)
            return s_acc, P, linv

        with scope("steady"):
            s_acc, P, linv = lax.fori_loop(1, NH, step, (jnp.zeros((8, D), f32), P, linv))

        o = None
        p = NH % 2
        for j in range(NS):
          with scope(f"L_{j // 8}"):
            jj = j + DQ
            if j >= NKV:
                A_cp(NH, j).wait()
            B_cp(NH, j).wait()
            if jj < NS:
                if jj >= NKV:
                    A_cp(NH, jj).start(priority=PA)
                B_cp(NH, jj).start(priority=PB)
            if j < NKV and (j + 1) % GPR == 0:
                o = v_compute(P, p, j // GPR, o)
        s8 = s_acc + out_proj(o, linv, p)
        s = jnp.sum(s8, axis=0, keepdims=True)
        if debug:
            o_ref[0:8, :] = jnp.broadcast_to(s, (8, D))
            o_ref[8:16, :] = gg
        else:
            out = x + s * gg[0:1]
            o_ref[...] = out.astype(o_ref.dtype)

    def fn(A_x, A_k_cache, A_v_cache, A_wq, A_wo, B_x, B_w_r, B_w_gate, B_w_up, B_w_down):
        hbm = pl.BlockSpec(memory_space=pltpu.HBM)
        oshape = jax.ShapeDtypeStruct((16, D), jnp.float32) if debug else jax.ShapeDtypeStruct((1, D), jnp.bfloat16)
        nP = (D * H * DH * 2) // GB + 3 * (-(-F // (GB // (D * 2))))
        out = pl.pallas_call(
            kernel, out_shape=oshape,
            in_specs=[hbm] * 9,
            out_specs=pl.BlockSpec(memory_space=pltpu.VMEM),
            scratch_shapes=[
                pltpu.VMEM((1, D), bf16), pltpu.VMEM((D,), bf16),
                pltpu.VMEM((D, H * DH), bf16), pltpu.VMEM((2, W, DH), bf16), pltpu.VMEM((2, W, DH), bf16),
                pltpu.VMEM((2, DH, D), bf16),
                pltpu.VMEM((F, D), bf16), pltpu.VMEM((F, D), bf16), pltpu.VMEM((F, D), bf16),
                pltpu.VMEM((H, 8, DH), f32),
                pltpu.SemaphoreType.DMA((2, NS)), pltpu.SemaphoreType.DMA((2, NS)), pltpu.SemaphoreType.DMA((nP,)), pltpu.SemaphoreType.DMA((2,))],
            compiler_params=pltpu.CompilerParams(vmem_limit_bytes=vlimit * 1024 * 1024, disable_bounds_checks=nobc, disable_semaphore_checks=nosc),
            name=name,
        )(A_x.reshape(1, D), A_k_cache, A_v_cache, A_wq, A_wo, B_w_r, B_w_gate.T, B_w_up.T, B_w_down)
        if debug:
            return out
        return out.reshape(1, 1, D)
    fn.__name__ = name
    return fn


_fn = make("recurrent_scan_decode", GD=128, DQ=40, GC=1024, nobc=True)


@jax.jit
def pallas_recurrent_scan__sliding_block_cached__moe_arch_mod__decode_kernel(
    A_x, A_k_cache, A_v_cache, A_wq, A_wo, B_x, B_w_r, B_w_gate, B_w_up, B_w_down,
):
    return _fn(A_x, A_k_cache, A_v_cache, A_wq, A_wo, B_x, B_w_r, B_w_gate, B_w_up, B_w_down)
```

```python
import functools
import jax, jax.numpy as jnp
from jax import lax
from jax.experimental import pallas as pl
from jax.experimental.pallas import tpu as pltpu
import numpy as np

H, SK, DH, W, D, F = 32, 32768, 128, 4096, 512, 1376
LOG2E = 1.4426950408889634
NT = (((1,), (1,)), ((), ()))
f32, bf16 = jnp.float32, jnp.bfloat16

NHS = 4
NSET = H // NHS
NM = 16
NU = 8
R = 64
FU = 32
NFU = F // FU


def make(name="v7", DM=6, debug=False, nobc=True, nosc=True, vlimit=64, scoped=False, skip=(), wq_sections=2, tail_order=1, tiny=False, ipos=8, ilv=0):
    assert 1 <= DM and NU * DM + 2 * NU <= R
    SC = (DH ** -0.5) * LOG2E
    scope = (lambda n: jax.named_scope(n)) if scoped else (lambda n: jax.named_scope("k"))
    NK = NSET * NM
    VOFF = NM - 1
    NIT = NK + NM

    def kernel(x_hbm, k_hbm, v_hbm, wq_hbm, wo_hbm, wr_hbm, wg_hbm, wu_hbm, wd_hbm, o_ref,
               xb, wrb, wqb, kr, vr, wob, wgb, wub, wdb, q_scr, p_scr, semA, semB, sem0):

        def mo(x, m):
            return x if isinstance(x, int) else pl.multiple_of(x, m)

        NQS = 64

        def semA_at(n, u):
            return semA.at[(NU * n + u) % R]

        def semB_at(n, u):
            return semB.at[(NU * n + u) % R]

        def K_cp(n, u):
            hd = NHS * (n // NM) + (u % NHS)
            t = (n % NM) + 16 * (u // NHS)
            slot = (NU * n + u) % R
            TR = 16 if tiny else 128
            return pltpu.make_async_copy(k_hbm.at[0, hd, pl.ds(mo(SK - W + t * 128, 128), TR), :], kr.at[slot, pl.ds(0, TR), :], semA_at(n, u))

        def V_cp(nv, u):
            hd = NHS * (nv // NM) + (u % NHS)
            t = (nv % NM) + 16 * (u // NHS)
            slot = (NU * nv + u) % R
            TR = 16 if (tiny and not (isinstance(nv, int) and nv >= NK + DM - VOFF)) else 128
            return pltpu.make_async_copy(v_hbm.at[0, hd, pl.ds(mo(SK - W + t * 128, 128), TR), :], vr.at[slot, pl.ds(0, TR), :], semB_at(nv + VOFF, u))

        def O_cp(w, sem):
            return pltpu.make_async_copy(wo_hbm.at[pl.ds(mo(w * FU, FU), FU), :], wob.at[pl.ds(mo(w * FU, FU), FU), :], sem)

        def F_cp(mat, i, sem):
            src, dst = ((wg_hbm, wgb), (wu_hbm, wub), (wd_hbm, wdb))[mat]
            return pltpu.make_async_copy(src.at[pl.ds(mo(i * FU, FU), FU), :], dst.at[pl.ds(mo(i * FU, FU), FU), :], sem)

        def Q_cp(i, sem):
            r8, c = i // 2, i % 2
            return pltpu.make_async_copy(wq_hbm.at[pl.ds(8 * r8, 8), pl.ds(c * 2048, 2048)], wqb.at[pl.ds(8 * r8, 8), pl.ds(c * 2048, 2048)], sem)
        spp = NQS // wq_sections
        qa = [(i % wq_sections) * spp + i // wq_sections for i in range(NQS)]
        qb_ = [NQS + (i % wq_sections) * spp + i // wq_sections for i in range(NQS)]

        def wo_early(n, u):
            return u * 15 + n

        ffn = []
        for c in range(11):
            for i in range(4 * c, min(4 * c + 4, NFU)):
                ffn.append((0, i)); ffn.append((1, i))
        wd_units = [(2, i) for i in range(NFU)]
        ffn += wd_units
        assert len(ffn) == 129
        lateA, lateB = {}, {}
        extraA = ffn[0]
        rest = ffn[1:]
        last_items = [("F",) + it for it in rest[-8:]]
        rest = rest[:-8]
        for idx, it in enumerate(rest):
            lateA[(NK + idx // NU, idx % NU)] = ("F",) + it
        wo_late = [("O", 120 + i) for i in range(8)]
        if tail_order == 0:
            for u in range(NU):
                lateA[(NIT - 1, u)] = last_items[u]
                lateB[(NIT - 1, u)] = wo_late[u]
        else:
            seq = wo_late + last_items
            for u in range(NU):
                lateA[(NIT - 1, u)] = seq[2 * u]
                lateB[(NIT - 1, u)] = seq[2 * u + 1]

        def late_cp(it, sem):
            return F_cp(it[1], it[2], sem) if it[0] == "F" else O_cp(it[1], sem)

        def A_static(n, u):
            if n < NK:
                return K_cp(n, u)
            return late_cp(lateA[(n, u)], semA_at(n, u))

        def B_static(n, u):
            if n < VOFF:
                return O_cp(wo_early(n, u), semB_at(n, u))
            if n < VOFF + NK:
                return V_cp(n - VOFF, u)
            return late_cp(lateB[(n, u)], semB_at(n, u))

        def A_pos(i):
            return Q_cp(qa[i], semA.at[i % R]) if i < NQS else A_static((i - NQS) // NU, (i - NQS) % NU)

        def B_pos(i):
            return Q_cp(qb_[i], semB.at[i % R]) if i < NQS else B_static((i - NQS) // NU, (i - NQS) % NU)
        issued = [0]
        DQ = DM * NU

        def issue_upto(n):
            while issued[0] < n:
                A_pos(issued[0]).start(priority=0)
                B_pos(issued[0]).start(priority=1)
                issued[0] += 1

        c_x = pltpu.make_async_copy(x_hbm, xb, sem0.at[0])
        c_wr = pltpu.make_async_copy(wr_hbm, wrb, sem0.at[1])
        c_x.start()
        c_wr.start()
        issue_upto(DQ)

        c_x.wait()
        x = xb[...].astype(f32).reshape(1, D)
        mean = jnp.mean(x, axis=-1, keepdims=True)
        xc = x - mean
        var = jnp.mean(xc * xc, axis=-1, keepdims=True)
        xn = xc / jnp.sqrt(var + 1e-5)
        xn_b1 = xn.astype(bf16)
        xn_b = jnp.broadcast_to(xn_b1, (8, D))
        c_wr.wait()
        r = jnp.sum(xn_b1.astype(f32) * wrb[...].astype(f32).reshape(1, D), axis=-1, keepdims=True)
        rs = jax.nn.sigmoid(r)

        rows = lax.broadcasted_iota(jnp.int32, (8, 128), 0)

        qacc = None
        arrived = set()
        qdone = set()
        QP = 4
        for i in range(NQS):
          with scope(f"Q_{i // 16}"):
            A_pos(i).wait(); B_pos(i).wait()
            arrived.add(qa[i]); arrived.add(qb_[i])
            issue_upto(i + 1 + DQ)
            for pp in range(QP):
                if pp not in qdone and all((32 * pp + j) in arrived for j in range(32)):
                    qdone.add(pp)
                    t = jnp.dot(xn_b[:, pp * 128:(pp + 1) * 128], wqb[pl.ds(pp * 128, 128), :], preferred_element_type=f32)
                    qacc = t if qacc is None else qacc + t
        for h in range(H):
            q_scr[h] = qacc[:, h * DH:(h + 1) * DH]

        def masks(m):
            return rows == m, rows == m - 8

        def k_region(n, S, m, C):
            m0, m1 = masks(m)
            C = list(C)
            for k in range(NHS):
                qb = q_scr[NHS * S + k].astype(bf16)
                for sec in range(2):
                    u = sec * NHS + k
                    s = lax.dot_general(qb, kr[(NU * n + u) % R], NT, preferred_element_type=f32)
                    i0 = 4 * k + 2 * sec
                    if isinstance(m, int):
                        if m < 8:
                            C[i0] = jnp.where(rows == m, s, C[i0])
                        else:
                            C[i0 + 1] = jnp.where(rows == m - 8, s, C[i0 + 1])
                    else:
                        C[i0] = jnp.where(m0, s, C[i0])
                        C[i0 + 1] = jnp.where(m1, s, C[i0 + 1])
            return C

        def v_region(nv, m, acc):
            m0, m1 = masks(m)
            acc = list(acc)
            for k in range(NHS):
                for sec in range(2):
                    u = sec * NHS + k
                    out = jnp.dot(p_scr[k, pl.ds(16 * sec, 16), :], vr[(NU * nv + u) % R], preferred_element_type=f32)
                    if isinstance(m, int):
                        sel = jnp.where(rows == m, out[0:8], 0.0) if m < 8 else jnp.where(rows == m - 8, out[8:16], 0.0)
                    else:
                        sel = jnp.where(m0, out[0:8], 0.0) + jnp.where(m1, out[8:16], 0.0)
                    acc[k] = acc[k] + sel
            return acc

        def softmax_set(C):
            linv = []
            for k in range(NHS):
                Cm = jnp.concatenate(C[4 * k:4 * k + 4], axis=0)
                mx = jnp.max(Cm, axis=(0, 1), keepdims=True)
                p = jnp.exp2((Cm - mx) * SC)
                l = jnp.sum(p, axis=(0, 1), keepdims=True)
                p_scr[k] = p.astype(bf16)
                linv.append(1.0 / l)
            return linv

        def normalize(acc, linv):
            return [(acc[k] * linv[k]).astype(bf16) for k in range(NHS)]

        def out_proj(on_k, h):
            return jnp.dot(on_k, wob[pl.ds(mo(h * DH, DH), DH), :], preferred_element_type=f32)

        zC = [jnp.zeros((8, 128), f32)] * 16
        zA = [jnp.zeros((8, 128), f32)] * NHS

        def late_dyn(n2, u):
            dn = n2 - NK
            j = u + 1
            mat = j % 2
            unit = 4 * (dn + j // 8) + (j % 8) // 2
            return F_cp(mat, unit, semA_at(n2, u))
        for dn in range(DM):
            for u in range(NU):
                j = u + 1
                assert lateA[(NK + dn, u)] == ("F", j % 2, 4 * (dn + j // 8) + (j % 8) // 2), (dn, u, lateA[(NK + dn, u)])

        def dyn_issue(n2, first, us=range(NU)):
            for u in us:
                if first:
                    K_cp(n2, u).start(priority=0)

                    @pl.when(n2 < VOFF)
                    def _():
                        O_cp(wo_early(n2, u), semB_at(n2, u)).start(priority=1)

                    @pl.when(n2 >= VOFF)
                    def _():
                        V_cp(n2 - VOFF, u).start(priority=1)
                else:
                    @pl.when(n2 < NK)
                    def _():
                        K_cp(n2, u).start(priority=0)

                    @pl.when(n2 >= NK)
                    def _():
                        late_dyn(n2, u).start(priority=0)
                    V_cp(n2 - VOFF, u).start(priority=1)

        extra_cp = F_cp(extraA[0], extraA[1], sem0.at[2])

        def iteration(n, S, m, C, acc, first):
            def wait_slot(u):
                K_cp(n, u).wait()
                pltpu.make_async_copy(vr.at[0], vr.at[0], semB_at(n, u)).wait()
            if ilv:
                for u in range(NU):
                    wait_slot(u)
                    dyn_issue(n + DM, first, [u])
            else:
                for u in range(ipos):
                    wait_slot(u)
                dyn_issue(n + DM, first)
                for u in range(ipos, NU):
                    wait_slot(u)
            if "kv" not in skip:
                if "k" not in skip:
                    C = k_region(n, S, m, C)
                if not first and "v" not in skip:
                    acc = v_region(n - NM, m, acc)
            return C, acc

        def body0(m, carry):
            C = iteration(m, 0, m, carry, None, True)[0]
            return tuple(C)
        with scope("set0"):
            C = lax.fori_loop(0, NM, body0, tuple(zC))
        linv = softmax_set(list(C))

        def set_body(S, carry):
            s_acc, linv = carry

            def body(m, cc):
                C, acc = iteration(S * NM + m, S, m, list(cc[0]), list(cc[1]), False)
                return tuple(C), tuple(acc)
            C, acc = lax.fori_loop(0, NM, body, (tuple(zC), tuple(zA)))
            on = normalize(acc, linv)
            for k in range(NHS):
                s_acc = s_acc + out_proj(on[k], NHS * (S - 1) + k)
            linv = softmax_set(list(C))
            return s_acc, tuple(linv)
        with scope("steady"):
            s_acc, linv = lax.fori_loop(1, NSET, set_body, (jnp.zeros((8, D), f32), tuple(linv)))

        issued[0] = NQS + (NK + DM) * NU
        acc = list(zA)
        st = dict(a=[None] * 11, y=None, on=None)
        got = set()
        done = set()
        extra_cp.start(priority=0)
        vdone = NK - NM

        def try_ffn():
            for c in range(11):
                us = range(4 * c, min(4 * c + 4, NFU))
                nr = len(list(us)) * FU
                if ("gu", c) not in done and all((0, i) in got and (1, i) in got for i in us):
                    done.add(("gu", c))
                    if "ffn" in skip:
                        st["a"][c] = jnp.zeros((8, nr), bf16)
                        continue
                    g = lax.dot_general(xn_b, wgb[pl.ds(128 * c, nr), :], NT, preferred_element_type=f32)
                    uu = lax.dot_general(xn_b, wub[pl.ds(128 * c, nr), :], NT, preferred_element_type=f32)
                    st["a"][c] = ((g * jax.nn.sigmoid(g)) * uu).astype(bf16)
                if ("d", c) not in done and ("gu", c) in done and all((2, i) in got for i in us):
                    done.add(("d", c))
                    if "ffn" in skip:
                        t = jnp.zeros((8, D), f32)
                    else:
                        t = jnp.dot(st["a"][c], wdb[pl.ds(128 * c, nr), :], preferred_element_type=f32)
                    st["y"] = t if st["y"] is None else st["y"] + t

        def try_oproj():
            nonlocal s_acc
            if st["on"] is None:
                return
            for k in range(NHS):
                h = H - NHS + k
                need = [w for w in range(4 * h, 4 * h + 4) if w >= 120]
                if ("o", k) not in done and all(("O", w) in got for w in need):
                    done.add(("o", k))
                    s_acc = s_acc + out_proj(st["on"][k], h)

        def mark(it):
            got.add((it[1], it[2]) if it[0] == "F" else it)

        for n in range(NK, NIT):
          with scope(f"L_{n - NK:02d}"):
            for u in range(NU):
                i = NQS + n * NU + u
                A_pos(i).wait(); B_pos(i).wait()
                mark(lateA[(n, u)])
                if (n, u) in lateB:
                    mark(lateB[(n, u)])
                if n == NK and u == NU - 1:
                    extra_cp.wait(); got.add(extraA)
                issue_upto(min(i + 1 + DQ, NQS + NIT * NU))
                fine = (n == NIT - 1)
                if u == NU - 1 or (fine and u % 2 == 1):
                    while vdone <= n - VOFF and vdone < NK and u == NU - 1:
                        if "kv" not in skip:
                            acc = v_region(vdone, vdone % NM, acc)
                        vdone += 1
                        if vdone == NK:
                            st["on"] = normalize(acc, linv)
                    try_ffn()
                    try_oproj()
        y = st["y"] * rs
        bb = xn + (xn * 0.0 + y)
        gg = bb * jax.nn.sigmoid(bb)
        s = jnp.sum(s_acc, axis=0, keepdims=True)
        if debug:
            o_ref[0:8, :] = jnp.broadcast_to(s, (8, D))
            o_ref[8:16, :] = gg
        else:
            out = x + s * gg[0:1]
            o_ref[...] = out.astype(o_ref.dtype)

    def fn(A_x, A_k_cache, A_v_cache, A_wq, A_wo, B_x, B_w_r, B_w_gate, B_w_up, B_w_down):
        hbm = pl.BlockSpec(memory_space=pltpu.HBM)
        oshape = jax.ShapeDtypeStruct((16, D), f32) if debug else jax.ShapeDtypeStruct((1, D), bf16)
        out = pl.pallas_call(
            kernel, out_shape=oshape,
            in_specs=[hbm] * 9,
            out_specs=pl.BlockSpec(memory_space=pltpu.VMEM),
            scratch_shapes=[
                pltpu.VMEM((1, D), bf16), pltpu.VMEM((D,), bf16),
                pltpu.VMEM((D, H * DH), bf16), pltpu.VMEM((R, 128, DH), bf16), pltpu.VMEM((R, 128, DH), bf16),
                pltpu.VMEM((H * DH, D), bf16),
                pltpu.VMEM((F, D), bf16), pltpu.VMEM((F, D), bf16), pltpu.VMEM((F, D), bf16),
                pltpu.VMEM((H, 8, DH), f32), pltpu.VMEM((NHS, 32, DH), bf16),
                pltpu.SemaphoreType.DMA((R,)), pltpu.SemaphoreType.DMA((R,)), pltpu.SemaphoreType.DMA((3,))],
            compiler_params=pltpu.CompilerParams(vmem_limit_bytes=vlimit * 1024 * 1024, disable_bounds_checks=nobc, disable_semaphore_checks=nosc),
            name=name,
        )(A_x.reshape(1, D), A_k_cache, A_v_cache, A_wq, A_wo, B_w_r, B_w_gate.T, B_w_up.T, B_w_down)
        if debug:
            return out
        return out.reshape(1, 1, D)
    fn.__name__ = name
    return fn


_fn = make("recurrent_scan_decode", DM=6, ipos=1)


@jax.jit
def pallas_recurrent_scan__sliding_block_cached__moe_arch_mod__decode_kernel(
    A_x, A_k_cache, A_v_cache, A_wq, A_wo, B_x, B_w_r, B_w_gate, B_w_up, B_w_down,
):
    return _fn(A_x, A_k_cache, A_v_cache, A_wq, A_wo, B_x, B_w_r, B_w_gate, B_w_up, B_w_down)
```

```python
import jax
import jax.numpy as jnp
from jax import lax
from jax.experimental import pallas as pl
from jax.experimental.pallas import tpu as pltpu

H, DH, W, D, F = 32, 128, 4096, 512, 1376
LOG2E = 1.4426950408889634
NT = (((1,), (1,)), ((), ()))
f32, bf16 = jnp.float32, jnp.bfloat16

NHS = 4
NSET = H // NHS
NM = 16
NU = 8
NK = NSET * NM
NQ = 8
FU = 32
NFU = F // FU
VOFF = 14
NIT = NK + NM
RS = 8
RV = 16


def make(name="v9", DM=6, debug=False, nobc=False, nosc=False, vlimit=64, scoped=False, skip=(), SK=32768, maxv=2, qsec=2, interpret=False):
    assert 1 <= DM <= RS - 1 and DM + 1 + (NM - VOFF) <= RV
    SC = (DH ** -0.5) * LOG2E
    scope = (lambda n: jax.named_scope(n)) if scoped else (lambda n: jax.named_scope("k"))
    NEARLY = VOFF * NU

    spp = 64 // qsec
    qa = [(i % qsec) * spp + i // qsec for i in range(64)]
    qb = [64 + v for v in qa]
    gu = []
    for c in range(11):
        for i in range(4 * c, min(4 * c + 4, NFU)):
            gu += [("F", 0, i), ("F", 1, i)]
    nwd_b = NU * (NM - VOFF - 1)
    aseq = gu + [("O", w) for w in range(NEARLY, 120)] + [("F", 2, i) for i in range(NFU - nwd_b)]
    assert len(aseq) == NM * NU + 1
    extraA, lateA = aseq[0], aseq[1:]
    lateB = [("F", 2, i) for i in range(NFU - nwd_b, NFU)] + [("O", 120 + i) for i in range(8)]
    assert len(lateB) == NU * (NM - VOFF)

    def kernel(x_hbm, k_hbm, v_hbm, wq_hbm, wo_hbm, wr_hbm, wg_hbm, wu_hbm, wd_hbm, o_ref,
               xb, wrb, wqb, kr, vr, wob, wgb, wub, wdb, q_scr, p_scr, semA, semB, sem0):

        def mo(x, m):
            return x if isinstance(x, int) else pl.multiple_of(x, m)

        def sA(it):
            return semA.at[it % RS]

        def sB(it):
            return semB.at[it % RS]

        def tile_src(src, hs, m, u):
            hd = NHS * hs + (u % NHS)
            t = m + 16 * (u // NHS)
            return src.at[0, hd, pl.ds(mo(SK - W + t * 128, 128), 128), :]

        def K_cp(n, u):
            return pltpu.make_async_copy(tile_src(k_hbm, n // NM, n % NM, u), kr.at[((NQ + n) % RS) * NU + u], sA(NQ + n))

        def V_cp(nv, u):
            return pltpu.make_async_copy(tile_src(v_hbm, nv // NM, nv % NM, u), vr.at[(nv % RV) * NU + u], sB(NQ + nv + VOFF))

        def O_cp(w, sem):
            return pltpu.make_async_copy(wo_hbm.at[pl.ds(mo(w * FU, FU), FU), :], wob.at[pl.ds(mo(w * FU, FU), FU), :], sem)

        def F_cp(mat, i, sem):
            src, dst = ((wg_hbm, wgb), (wu_hbm, wub), (wd_hbm, wdb))[mat]
            return pltpu.make_async_copy(src.at[pl.ds(mo(i * FU, FU), FU), :], dst.at[pl.ds(mo(i * FU, FU), FU), :], sem)

        def Q_cp(i, sem):
            r8, c = i // 2, i % 2
            return pltpu.make_async_copy(wq_hbm.at[pl.ds(8 * r8, 8), pl.ds(c * 2048, 2048)], wqb.at[pl.ds(8 * r8, 8), pl.ds(c * 2048, 2048)], sem)

        def late_cp(it, sem):
            return F_cp(it[1], it[2], sem) if it[0] == "F" else O_cp(it[1], sem)

        def wait_iter(it):
            d = kr.at[pl.ds(0, NU)]
            pltpu.make_async_copy(d, d, sA(it)).wait()
            pltpu.make_async_copy(d, d, sB(it)).wait()

        def issue_static(it):
            n = it - NQ
            for u in range(NU):
                if it < NQ:
                    a, b = Q_cp(qa[it * NU + u], sA(it)), Q_cp(qb[it * NU + u], sB(it))
                else:
                    a = K_cp(n, u) if n < NK else late_cp(lateA[(n - NK) * NU + u], sA(it))
                    if n < VOFF:
                        b = O_cp(u * VOFF + n, sB(it))
                    elif n < VOFF + NK:
                        b = V_cp(n - VOFF, u)
                    else:
                        b = late_cp(lateB[(n - VOFF - NK) * NU + u], sB(it))
                a.start(priority=0)
                b.start(priority=1)

        c_x = pltpu.make_async_copy(x_hbm, xb, sem0.at[0])
        c_wr = pltpu.make_async_copy(wr_hbm, wrb, sem0.at[1])
        c_x.start()
        c_wr.start()
        for it in range(DM):
            issue_static(it)

        c_x.wait()
        x = xb[...].astype(f32).reshape(1, D)
        mean = jnp.mean(x, axis=-1, keepdims=True)
        xc = x - mean
        var = jnp.mean(xc * xc, axis=-1, keepdims=True)
        xn = xc / jnp.sqrt(var + 1e-5)
        xn_b1 = xn.astype(bf16)
        xn_b = jnp.broadcast_to(xn_b1, (8, D))
        c_wr.wait()
        r = jnp.sum(xn_b1.astype(f32) * wrb[...].astype(f32).reshape(1, D), axis=-1, keepdims=True)
        rs = jax.nn.sigmoid(r)
        rows = lax.broadcasted_iota(jnp.int32, (8, 128), 0)

        qacc = None
        arrived, qdone = set(), set()
        for it in range(NQ):
          with scope(f"Q_{it}"):
            issue_static(it + DM)
            wait_iter(it)
            arrived.update(qa[it * NU:(it + 1) * NU]); arrived.update(qb[it * NU:(it + 1) * NU])
            for pp in range(4):
                if pp not in qdone and all((32 * pp + j) in arrived for j in range(32)):
                    qdone.add(pp)
                    t = jnp.dot(xn_b[:, pp * 128:(pp + 1) * 128], wqb[pl.ds(pp * 128, 128), :], preferred_element_type=f32)
                    qacc = t if qacc is None else qacc + t
        for h in range(H):
            q_scr[h] = qacc[:, h * DH:(h + 1) * DH]

        def k_region(n, S, m, C):
            C = list(C)
            base = ((NQ + n) % RS) * NU
            for k in range(NHS):
                qv = q_scr[NHS * S + k].astype(bf16)
                for sec in range(2):
                    s = lax.dot_general(qv, kr[base + sec * NHS + k], NT, preferred_element_type=f32)
                    i0 = 4 * k + 2 * sec
                    if isinstance(m, int):
                        i1, rr = (i0, m) if m < 8 else (i0 + 1, m - 8)
                        C[i1] = jnp.where(rows == rr, s, C[i1])
                    else:
                        C[i0] = jnp.where(rows == m, s, C[i0])
                        C[i0 + 1] = jnp.where(rows == m - 8, s, C[i0 + 1])
            return C

        def v_region(nv, m, acc):
            acc = list(acc)
            base = (nv % RV) * NU
            for k in range(NHS):
                for sec in range(2):
                    out = jnp.dot(p_scr[k, pl.ds(16 * sec, 16), :], vr[base + sec * NHS + k], preferred_element_type=f32)
                    if isinstance(m, int):
                        sel = jnp.where(rows == m, out[0:8], 0.0) if m < 8 else jnp.where(rows == m - 8, out[8:16], 0.0)
                    else:
                        sel = jnp.where(rows == m, out[0:8], 0.0) + jnp.where(rows == m - 8, out[8:16], 0.0)
                    acc[k] = acc[k] + sel
            return acc

        def softmax_set(C):
            linv = []
            for k in range(NHS):
                Cm = jnp.concatenate(C[4 * k:4 * k + 4], axis=0)
                mx = jnp.max(Cm, axis=(0, 1), keepdims=True)
                p = jnp.exp2((Cm - mx) * SC)
                l = jnp.sum(p, axis=(0, 1), keepdims=True)
                p_scr[k] = p.astype(bf16)
                linv.append(1.0 / l)
            return linv

        def normalize(acc, linv):
            return [jnp.broadcast_to(jnp.sum(acc[k], axis=0, keepdims=True) * linv[k], (8, DH)).astype(bf16) for k in range(NHS)]

        def out_proj(on_k, h):
            return jnp.dot(on_k, wob[pl.ds(mo(h * DH, DH), DH), :], preferred_element_type=f32)

        zC = [jnp.zeros((8, 128), f32)] * 16
        zA = [jnp.zeros((8, 128), f32)] * NHS
        for dn in range(DM):
            for u in range(NU):
                j = u + 1
                assert lateA[dn * NU + u] == ("F", j % 2, 4 * (dn + j // 8) + (j % 8) // 2)

        def dyn_issue(n2, first):
            for u in range(NU):
                if first:
                    K_cp(n2, u).start(priority=0)

                    @pl.when(n2 < VOFF)
                    def _():
                        O_cp(u * VOFF + n2, sB(NQ + n2)).start(priority=1)

                    @pl.when(n2 >= VOFF)
                    def _():
                        V_cp(n2 - VOFF, u).start(priority=1)
                else:
                    @pl.when(n2 < NK)
                    def _():
                        K_cp(n2, u).start(priority=0)

                    @pl.when(n2 >= NK)
                    def _():
                        j = u + 1
                        F_cp(j % 2, 4 * (n2 - NK + j // 8) + (j % 8) // 2, sA(NQ + n2)).start(priority=0)
                    V_cp(n2 - VOFF, u).start(priority=1)

        def iteration(n, S, m, C, acc, first):
            dyn_issue(n + DM, first)
            wait_iter(NQ + n)
            if "kv" not in skip:
                C = k_region(n, S, m, C)
                if not first:
                    acc = v_region(n - NM, m, acc)
            return C, acc

        def body0(m, carry):
            return tuple(iteration(m, 0, m, carry, None, True)[0])
        with scope("set0"):
            C = lax.fori_loop(0, NM, body0, tuple(zC))
        linv = softmax_set(list(C))

        def set_body(S, carry):
            s_acc, linv = carry

            def body(m, cc):
                C, acc = iteration(S * NM + m, S, m, list(cc[0]), list(cc[1]), False)
                return tuple(C), tuple(acc)
            C, acc = lax.fori_loop(0, NM, body, (tuple(zC), tuple(zA)))
            on = normalize(acc, linv)
            for k in range(NHS):
                s_acc = s_acc + out_proj(on[k], NHS * (S - 1) + k)
            return s_acc, tuple(softmax_set(list(C)))
        with scope("steady"):
            s_acc, linv = lax.fori_loop(1, NSET, set_body, (jnp.zeros((8, D), f32), tuple(linv)))

        acc = list(zA)
        st = dict(a=[None] * 11, y=None, on=None)
        got, done = set(), set()
        extra_cp = late_cp(extraA, sem0.at[2])
        extra_cp.start(priority=0)
        vdone = NK - NM

        def try_ffn():
            for c in range(11):
                us = range(4 * c, min(4 * c + 4, NFU))
                nr = len(us) * FU
                if ("gu", c) not in done and all(("F", 0, i) in got and ("F", 1, i) in got for i in us):
                    done.add(("gu", c))
                    if "ffn" in skip:
                        st["a"][c] = jnp.zeros((8, nr), bf16)
                    else:
                        g = lax.dot_general(xn_b, wgb[pl.ds(128 * c, nr), :], NT, preferred_element_type=f32)
                        uu = lax.dot_general(xn_b, wub[pl.ds(128 * c, nr), :], NT, preferred_element_type=f32)
                        st["a"][c] = ((g * jax.nn.sigmoid(g)) * uu).astype(bf16)
                if ("d", c) not in done and ("gu", c) in done and all(("F", 2, i) in got for i in us):
                    done.add(("d", c))
                    t = jnp.zeros((8, D), f32) if "ffn" in skip else jnp.dot(st["a"][c], wdb[pl.ds(128 * c, nr), :], preferred_element_type=f32)
                    st["y"] = t if st["y"] is None else st["y"] + t
            if "gg" not in st and all(("d", c) in done for c in range(11)):
                bb = xn + (xn * 0.0 + st["y"] * rs)
                st["gg"] = bb * jax.nn.sigmoid(bb)

        def try_oproj():
            nonlocal s_acc
            if st["on"] is None:
                return
            for k in range(NHS):
                h = H - NHS + k
                if ("o", k) not in done and all(("O", w) in got for w in range(4 * h, 4 * h + 4) if w >= NEARLY):
                    done.add(("o", k))
                    s_acc = s_acc + out_proj(st["on"][k], h)

        for n in range(NK, NIT):
          with scope(f"L_{n - NK:02d}"):
            if n + DM < NIT:
                issue_static(NQ + n + DM)
            wait_iter(NQ + n)
            got.update(lateA[(n - NK) * NU:(n - NK + 1) * NU])
            if n >= VOFF + NK:
                got.update(lateB[(n - VOFF - NK) * NU:(n - VOFF - NK + 1) * NU])
            if n == NK:
                extra_cp.wait()
                got.add(extraA)
            nreg = 0
            while vdone <= n - VOFF and vdone < NK and (nreg < maxv or n >= VOFF + NK - 1):
                if "kv" not in skip:
                    acc = v_region(vdone, vdone % NM, acc)
                vdone += 1
                nreg += 1
                if vdone == NK:
                    st["on"] = normalize(acc, linv)
            try_ffn()
            try_oproj()
        assert vdone == NK and all(("o", k) in done for k in range(NHS)) and "gg" in st
        gg = st["gg"]
        s = s_acc[0:1]
        if debug:
            o_ref[0:8, :] = jnp.broadcast_to(s, (8, D))
            o_ref[8:16, :] = gg
        else:
            o_ref[...] = (x + s * gg[0:1]).astype(o_ref.dtype)

    def fn(A_x, A_k_cache, A_v_cache, A_wq, A_wo, B_x, B_w_r, B_w_gate, B_w_up, B_w_down):
        hbm = pl.BlockSpec(memory_space=pltpu.HBM)
        oshape = jax.ShapeDtypeStruct((16, D), f32) if debug else jax.ShapeDtypeStruct((1, D), bf16)
        out = pl.pallas_call(
            kernel, out_shape=oshape,
            in_specs=[hbm] * 9,
            out_specs=pl.BlockSpec(memory_space=pltpu.VMEM),
            scratch_shapes=[
                pltpu.VMEM((1, D), bf16), pltpu.VMEM((D,), bf16),
                pltpu.VMEM((D, H * DH), bf16), pltpu.VMEM((RS * NU, 128, DH), bf16), pltpu.VMEM((RV * NU, 128, DH), bf16),
                pltpu.VMEM((H * DH, D), bf16),
                pltpu.VMEM((F, D), bf16), pltpu.VMEM((F, D), bf16), pltpu.VMEM((F, D), bf16),
                pltpu.VMEM((H, 8, DH), f32), pltpu.VMEM((NHS, 32, DH), bf16),
                pltpu.SemaphoreType.DMA((RS,)), pltpu.SemaphoreType.DMA((RS,)), pltpu.SemaphoreType.DMA((3,))],
            compiler_params=pltpu.CompilerParams(vmem_limit_bytes=vlimit * 1024 * 1024, disable_bounds_checks=nobc, disable_semaphore_checks=nosc),
            name=name, interpret=interpret,
        )(A_x.reshape(1, D), A_k_cache, A_v_cache, A_wq, A_wo, B_w_r, B_w_gate.T, B_w_up.T, B_w_down)
        return out if debug else out.reshape(1, 1, D)
    fn.__name__ = name
    return fn


_fn = make("recurrent_scan_decode", DM=6, nosc=True)


@jax.jit
def pallas_recurrent_scan__sliding_block_cached__moe_arch_mod__decode_kernel(
    A_x, A_k_cache, A_v_cache, A_wq, A_wo, B_x, B_w_r, B_w_gate, B_w_up, B_w_down,
):
    return _fn(A_x, A_k_cache, A_v_cache, A_wq, A_wo, B_x, B_w_r, B_w_gate, B_w_up, B_w_down)
```

```python
import math

import jax
import jax.numpy as jnp
from jax import lax
from jax.experimental import pallas as pl
from jax.experimental.pallas import tpu as pltpu

F32, BF16 = jnp.float32, jnp.bfloat16

H, DH, W, D, FF = 32, 128, 4096, 512, 1376
NT = (((1,), (1,)), ((), ()))

NHS = 4
NSET = H // NHS
NM = 16
NU = 8
NQ = 8
NK = NSET * NM
FU = 32
NFU = FF // FU
DM = 6
RS = 8
RV = 16
VOFF = 12
NEARLY = VOFF * NU
NB_END = VOFF + NK + 2
SKEW = 4

_QA = [(i % 2) * 32 + i // 2 for i in range(64)]
_QB = [64 + i for i in _QA]
_GU = [("F", m, i) for c in range(11) for i in range(4 * c, min(4 * c + 4, NFU)) for m in (0, 1)]
_A_TAIL = _GU + [("O", w) for w in range(NEARLY, 120)] + [("F", 2, i) for i in range(NFU - NU)]
_EXTRA, _LATE_A = _A_TAIL[0], _A_TAIL[1:]
_LATE_B = [("F", 2, i) for i in range(NFU - NU, NFU)] + [("O", w) for w in range(120, 128)]
NA_END = NK + len(_LATE_A) // NU
assert len(_LATE_A) % NU == 0 and len(_LATE_B) == 2 * NU
assert DM < RS and DM + 1 + (NM - VOFF) <= RV and SKEW < DM and NA_END <= NB_END + SKEW


def _late_a_lookahead(dn, u):
    j = u + 1
    return j % 2, 4 * (dn + j // 8) + (j % 8) // 2


assert all(_LATE_A[dn * NU + u] == ("F",) + _late_a_lookahead(dn, u)
           for dn in range(DM) for u in range(NU))


def _decode_kernel(x_hbm, k_hbm, v_hbm, wq_hbm, wo_hbm, wr_hbm, wg_hbm, wu_hbm, wd_hbm, o_ref,
                   xb, wrb, wqb, kr, vr, wob, wgb, wub, wdb, q_scr, p_scr, sem_a, sem_b, sem_x):
    sk = k_hbm.shape[2]
    score_scale = (DH ** -0.5) * math.log2(math.e)

    def aligned(i, m):
        return i if isinstance(i, int) else pl.multiple_of(i, m)

    def sa(it):
        return sem_a.at[it % RS]

    def sb(it):
        return sem_b.at[it % RS]

    def kv_tile(src, j, u):
        row = sk - W + ((j % NM) + NM * (u // NHS)) * 128
        return src.at[0, NHS * (j // NM) + u % NHS, pl.ds(aligned(row, 128), 128), :]

    def k_slot(n):
        return ((NQ + n) % RS) * NU

    def v_slot(j):
        return (j % RV) * NU

    def k_copy(n, u):
        return pltpu.make_async_copy(kv_tile(k_hbm, n, u), kr.at[k_slot(n) + u], sa(NQ + n))

    def v_copy(j, u):
        return pltpu.make_async_copy(kv_tile(v_hbm, j, u), vr.at[v_slot(j) + u], sb(NQ + VOFF + j))

    def row_copy(src, dst, i, sem):
        rows = pl.ds(aligned(i * FU, FU), FU)
        return pltpu.make_async_copy(src.at[rows, :], dst.at[rows, :], sem)

    def wq_copy(i, sem):
        r, c = pl.ds(8 * (i // 2), 8), pl.ds(2048 * (i % 2), 2048)
        return pltpu.make_async_copy(wq_hbm.at[r, c], wqb.at[r, c], sem)

    def tail_copy(item, sem):
        if item[0] == "O":
            return row_copy(wo_hbm, wob, item[1], sem)
        src, dst = ((wg_hbm, wgb), (wu_hbm, wub), (wd_hbm, wdb))[item[1]]
        return row_copy(src, dst, item[2], sem)

    def a_copy(it, u):
        n = it - NQ
        if n < 0:
            return wq_copy(_QA[it * NU + u], sa(it))
        if n < NK:
            return k_copy(n, u)
        return tail_copy(_LATE_A[(n - NK) * NU + u], sa(it))

    def b_copy(it, u):
        n = it - NQ
        if n < 0:
            return wq_copy(_QB[it * NU + u], sb(it))
        if n < VOFF:
            return row_copy(wo_hbm, wob, u * VOFF + n, sb(it))
        if n < VOFF + NK:
            return v_copy(n - VOFF, u)
        item = _LATE_B[(n - VOFF - NK) * NU + u]
        if item[0] == "O" and item[1] >= 124:
            return row_copy(wo_hbm, wob, item[1], sem_x.at[3 + item[1] - 124])
        return tail_copy(item, sb(it))

    def issue(it):
        n = it - NQ
        for u in range(NU):
            if n < NA_END:
                a_copy(it, u).start(priority=0)
            if n < NB_END:
                b_copy(it, u).start(priority=1)

    def wait_tiles(ring, slot, sem):
        region = ring.at[pl.ds(slot, NU)]
        pltpu.make_async_copy(region, region, sem).wait()

    x_copy = pltpu.make_async_copy(x_hbm, xb, sem_x.at[0])
    wr_copy = pltpu.make_async_copy(wr_hbm, wrb, sem_x.at[1])
    x_copy.start()
    wr_copy.start()
    for it in range(DM):
        issue(it)

    x_copy.wait()
    x = xb[...].astype(F32)
    xc = x - jnp.mean(x, axis=-1, keepdims=True)
    xn = xc / jnp.sqrt(jnp.mean(xc * xc, axis=-1, keepdims=True) + 1e-5)
    xn_row = xn.astype(BF16)
    xn_lhs = jnp.broadcast_to(xn_row, (8, D))
    wr_copy.wait()
    r = jnp.sum(xn_row.astype(F32) * wrb[...].astype(F32).reshape(1, D), axis=-1, keepdims=True)
    r_gate = jax.nn.sigmoid(r)
    rows = lax.broadcasted_iota(jnp.int32, (8, 128), 0)

    q = None
    landed, slabs = set(), set()
    for it in range(NQ):
        issue(it + DM)
        for u in range(NU):
            a_copy(it, u).wait()
            b_copy(it, u).wait()
        landed.update(_QA[it * NU:(it + 1) * NU] + _QB[it * NU:(it + 1) * NU])
        for s in range(D // 128):
            if s not in slabs and all(32 * s + j in landed for j in range(32)):
                slabs.add(s)
                t = jnp.dot(xn_lhs[:, s * 128:(s + 1) * 128], wqb[pl.ds(s * 128, 128), :],
                            preferred_element_type=F32)
                q = t if q is None else q + t
    for h in range(H):
        q_scr[h] = q[:, h * DH:(h + 1) * DH]

    def score_tiles(n, s_idx, m, sc):
        sc = list(sc)
        base = k_slot(n)
        for k in range(NHS):
            qv = q_scr[NHS * s_idx + k].astype(BF16)
            for half in range(2):
                t = lax.dot_general(qv, kr[base + half * NHS + k], NT, preferred_element_type=F32)
                i = 4 * k + 2 * half
                sc[i] = jnp.where(rows == m, t, sc[i])
                sc[i + 1] = jnp.where(rows == m - 8, t, sc[i + 1])
        return sc

    def weighted_tiles(j, m, acc):
        acc = list(acc)
        base = v_slot(j)
        for k in range(NHS):
            for half in range(2):
                t = jnp.dot(p_scr[k, pl.ds(16 * half, 16), :], vr[base + half * NHS + k],
                            preferred_element_type=F32)
                if isinstance(m, int):
                    part = t[0:8] if m < 8 else t[8:16]
                    acc[k] = acc[k] + jnp.where(rows == m % 8, part, 0.0)
                else:
                    acc[k] = acc[k] + (jnp.where(rows == m, t[0:8], 0.0)
                                       + jnp.where(rows == m - 8, t[8:16], 0.0))
        return acc

    def softmax_set(sc):
        inv = []
        for k in range(NHS):
            c = jnp.concatenate(sc[4 * k:4 * k + 4], axis=0)
            p = jnp.exp2((c - jnp.max(c, axis=(0, 1), keepdims=True)) * score_scale)
            p_scr[k] = p.astype(BF16)
            inv.append(1.0 / jnp.sum(p, axis=(0, 1), keepdims=True))
        return tuple(inv)

    def normalize(acc, inv):
        return [jnp.broadcast_to(jnp.sum(acc[k], axis=0, keepdims=True) * inv[k], (8, DH)).astype(BF16)
                for k in range(NHS)]

    def out_proj(o_head, h):
        return jnp.dot(o_head, wob[pl.ds(aligned(h * DH, DH), DH), :], preferred_element_type=F32)

    zero_scores = (jnp.zeros((8, 128), F32),) * (4 * NHS)
    zero_acc = (jnp.zeros((8, 128), F32),) * NHS

    def first_set_step(m, sc):
        n2 = m + DM
        for u in range(NU):
            k_copy(n2, u).start(priority=0)

            @pl.when(n2 < VOFF)
            def _():
                row_copy(wo_hbm, wob, u * VOFF + n2, sb(NQ + n2)).start(priority=1)

            @pl.when(n2 >= VOFF)
            def _():
                v_copy(n2 - VOFF, u).start(priority=1)

        wait_tiles(kr, k_slot(m), sa(NQ + m))

        @pl.when(m < VOFF)
        def _():
            for u in range(NU):
                row_copy(wo_hbm, wob, u * VOFF + m, sb(NQ + m)).wait()

        @pl.when(m >= VOFF)
        def _():
            wait_tiles(vr, v_slot(m - VOFF), sb(NQ + m))

        return tuple(score_tiles(m, 0, m, sc))

    inv = softmax_set(list(lax.fori_loop(0, NM, first_set_step, zero_scores)))

    def run_set(s_idx):
        def step(m, carry):
            n = s_idx * NM + m
            n2 = n + DM
            for u in range(NU):
                @pl.when(n2 < NK)
                def _():
                    k_copy(n2, u).start(priority=0)

                @pl.when(n2 >= NK)
                def _():
                    mat, unit = _late_a_lookahead(n2 - NK, u)
                    tail_copy(("F", mat, unit), sa(NQ + n2)).start(priority=0)

                v_copy(n2 - VOFF, u).start(priority=1)
            wait_tiles(kr, k_slot(n), sa(NQ + n))
            wait_tiles(vr, v_slot(n - VOFF), sb(NQ + n))
            sc = score_tiles(n, s_idx, m, carry[0])
            acc = weighted_tiles(n - NM, m, carry[1])
            return tuple(sc), tuple(acc)
        return lax.fori_loop(0, NM, step, (zero_scores, zero_acc))

    def set_step(s_idx, carry):
        s_acc, inv_prev = carry
        sc, acc = run_set(s_idx)
        o_set = normalize(acc, inv_prev)
        for k in range(NHS):
            s_acc = s_acc + out_proj(o_set[k], NHS * (s_idx - 1) + k)
        return s_acc, softmax_set(list(sc))

    s_acc, inv = lax.fori_loop(1, NSET - 1, set_step, (jnp.zeros((8, D), F32), inv))
    sc, acc = run_set(NSET - 1)
    pending = [(o, NHS * (NSET - 2) + k) for k, o in enumerate(normalize(acc, inv))]
    inv = softmax_set(list(sc))

    extra_copy = tail_copy(_EXTRA, sem_x.at[2])
    extra_copy.start(priority=0)
    acc = list(zero_acc)
    v_next, a_next = NK - NM, NK
    have, act, y, gate, o_last = set(), {}, None, None, None
    for n in range(NK, NB_END):
        last = n == NB_END - 1
        issue(NQ + n + DM)
        while a_next < NA_END and (a_next <= n + SKEW or last):
            for u in range(NU):
                a_copy(NQ + a_next, u).wait()
            have.update(_LATE_A[(a_next - NK) * NU:(a_next - NK + 1) * NU])
            a_next += 1
        if n == NK:
            extra_copy.wait()
            have.add(_EXTRA)
        if n < VOFF + NK:
            wait_tiles(vr, v_slot(n - VOFF), sb(NQ + n))
        else:
            for u in range(NU // 2 if last else NU):
                b_copy(NQ + n, u).wait()
                have.add(_LATE_B[(n - VOFF - NK) * NU + u])

        budget = NM if n == VOFF + NK - 1 else 2
        while v_next <= min(n - VOFF, NK - 1) and budget > 0:
            acc = weighted_tiles(v_next, v_next % NM, acc)
            v_next, budget = v_next + 1, budget - 1
            if v_next == NK:
                o_set = normalize(acc, inv)
                pending += [(o_set[k], H - NHS + k) for k in range(NHS - 1)]
                o_last = o_set[NHS - 1]

        for c in range(11):
            units = range(4 * c, min(4 * c + 4, NFU))
            chunk = pl.ds(128 * c, FU * len(units))
            if c not in act and all(("F", m, i) in have for m in (0, 1) for i in units):
                g = lax.dot_general(xn_lhs, wgb[chunk, :], NT, preferred_element_type=F32)
                up = lax.dot_general(xn_lhs, wub[chunk, :], NT, preferred_element_type=F32)
                act[c] = ((g * jax.nn.sigmoid(g)) * up).astype(BF16)
            if act.get(c) is not None and all(("F", 2, i) in have for i in units):
                t = jnp.dot(act[c], wdb[chunk, :], preferred_element_type=F32)
                y = t if y is None else y + t
                act[c] = None
        if gate is None and len(act) == 11 and all(a is None for a in act.values()):
            routed = xn + (xn * 0.0 + y * r_gate)
            gate = routed * jax.nn.sigmoid(routed)

        for o_head, h in list(pending):
            if all(("O", w) in have for w in range(4 * h, 4 * h + 4)):
                s_acc = s_acc + out_proj(o_head, h)
                pending.remove((o_head, h))
    assert v_next == NK and a_next == NA_END and gate is not None and not pending

    o_col = jnp.transpose(jnp.broadcast_to(o_last.astype(F32)[0:1], (DH, DH)))
    part = None
    for j in range(4):
        row_copy(wo_hbm, wob, 124 + j, sem_x.at[3 + j]).wait()
        prod = wob[pl.ds((124 + j) * FU, FU), :].astype(F32) * jnp.concatenate(
            [o_col[j * FU:(j + 1) * FU]] * (D // 128), axis=1)
        for i in range(FU // 8):
            blk = prod[8 * i:8 * i + 8]
            part = blk if part is None else part + blk
    s = s_acc[0:1] + jnp.sum(part, axis=0, keepdims=True)

    o_ref[...] = (x + s * gate[0:1]).astype(o_ref.dtype)


@jax.jit
def pallas_recurrent_scan__sliding_block_cached__moe_arch_mod__decode_kernel(
    A_x: jax.Array,
    A_k_cache: jax.Array,
    A_v_cache: jax.Array,
    A_wq: jax.Array,
    A_wo: jax.Array,
    B_x: jax.Array,
    B_w_r: jax.Array,
    B_w_gate: jax.Array,
    B_w_up: jax.Array,
    B_w_down: jax.Array,
):
    del B_x
    assert A_x.shape == (1, 1, D) and A_k_cache.shape[:2] == (1, H) and A_k_cache.shape[3] == DH
    assert min(4096, max(256, A_k_cache.shape[2] // 4)) == W and A_k_cache.shape[2] % 128 == 0
    in_hbm = pl.BlockSpec(memory_space=pltpu.HBM)
    out = pl.pallas_call(
        _decode_kernel,
        out_shape=jax.ShapeDtypeStruct((1, D), A_x.dtype),
        in_specs=[in_hbm] * 9,
        out_specs=pl.BlockSpec(memory_space=pltpu.VMEM),
        scratch_shapes=[
            pltpu.VMEM((1, D), BF16),
            pltpu.VMEM((D,), BF16),
            pltpu.VMEM((D, H * DH), BF16),
            pltpu.VMEM((RS * NU, 128, DH), BF16),
            pltpu.VMEM((RV * NU, 128, DH), BF16),
            pltpu.VMEM((H * DH, D), BF16),
            pltpu.VMEM((FF, D), BF16),
            pltpu.VMEM((FF, D), BF16),
            pltpu.VMEM((FF, D), BF16),
            pltpu.VMEM((H, 8, DH), F32),
            pltpu.VMEM((NHS, 32, DH), BF16),
            pltpu.SemaphoreType.DMA((RS,)),
            pltpu.SemaphoreType.DMA((RS,)),
            pltpu.SemaphoreType.DMA((7,)),
        ],
        compiler_params=pltpu.CompilerParams(
            vmem_limit_bytes=48 * 1024 * 1024,
            disable_semaphore_checks=True,
        ),
        name="recurrent_scan_decode",
    )(
        A_x.reshape(1, D), A_k_cache, A_v_cache, A_wq, A_wo, B_w_r,
        B_w_gate.T, B_w_up.T, B_w_down,
    )
    return out.reshape(1, 1, D)
```

```python
import math

import jax
import jax.numpy as jnp
from jax import lax
from jax.experimental import pallas as pl
from jax.experimental.pallas import tpu as pltpu

F32, BF16 = jnp.float32, jnp.bfloat16

H, DH, W, D, FF = 32, 128, 4096, 512, 1376
NT = (((1,), (1,)), ((), ()))

NHS = 4
NSET = H // NHS
NM = 16
NU = 8
NQ = 8
NK = NSET * NM
FU = 32
NFU = FF // FU
DM = 6
RS = 8
RV = 16
VOFF = 12
NEARLY = VOFF * NU
NB_END = VOFF + NK + 2
SKEW = 4

_QA = [(i % 2) * 32 + i // 2 for i in range(64)]
_QB = [64 + i for i in _QA]
_GU = [("F", m, i) for c in range(11) for i in range(4 * c, min(4 * c + 4, NFU)) for m in (0, 1)]
_A_TAIL = _GU + [("O", w) for w in range(NEARLY, 120)] + [("F", 2, i) for i in range(NFU - NU)]
_EXTRA, _LATE_A = _A_TAIL[0], _A_TAIL[1:]
_LATE_B = [("F", 2, i) for i in range(NFU - NU, NFU)] + [("O", w) for w in range(120, 128)]
NA_END = NK + len(_LATE_A) // NU
assert len(_LATE_A) % NU == 0 and len(_LATE_B) == 2 * NU
assert DM < RS and DM + 1 + (NM - VOFF) <= RV and SKEW < DM and NA_END <= NB_END + SKEW


def _late_a_lookahead(dn, u):
    j = u + 1
    return j % 2, 4 * (dn + j // 8) + (j % 8) // 2


assert all(_LATE_A[dn * NU + u] == ("F",) + _late_a_lookahead(dn, u)
           for dn in range(DM) for u in range(NU))


def _decode_kernel(x_hbm, k_hbm, v_hbm, wq_hbm, wo_hbm, wr_hbm, wg_hbm, wu_hbm, wd_hbm, o_ref,
                   xb, wrb, wqb, kr, vr, wob, wgb, wub, wdb, q_scr, p_scr, sem_a, sem_b, sem_x):
    sk = k_hbm.shape[2]
    score_scale = (DH ** -0.5) * math.log2(math.e)

    def aligned(i, m):
        return i if isinstance(i, int) else pl.multiple_of(i, m)

    def sa(it):
        return sem_a.at[it % RS]

    def sb(it):
        return sem_b.at[it % RS]

    def kv_copy(src, ring, slot, sem, j, u):
        pair, half, blk = u % 2, (u // 2) % 2, u // 4
        heads = pl.ds(aligned(NHS * (j // NM) + 2 * pair, 2), 2)
        keys = pl.ds(aligned(sk - W + ((j % NM) + NM * half) * 128 + 64 * blk, 64), 64)
        return pltpu.make_async_copy(
            src.at[0, heads, keys, :],
            ring.at[slot + half, pl.ds(2 * pair, 2), pl.ds(64 * blk, 64), :], sem)

    def k_slot(n):
        return ((NQ + n) % RS) * 2

    def v_slot(j):
        return (j % RV) * 2

    def k_copy(n, u):
        return kv_copy(k_hbm, kr, k_slot(n), sa(NQ + n), n, u)

    def v_copy(j, u):
        return kv_copy(v_hbm, vr, v_slot(j), sb(NQ + VOFF + j), j, u)

    def row_copy(src, dst, i, sem):
        rows = pl.ds(aligned(i * FU, FU), FU)
        return pltpu.make_async_copy(src.at[rows, :], dst.at[rows, :], sem)

    def wq_copy(i, sem):
        r, c = pl.ds(8 * (i // 2), 8), pl.ds(2048 * (i % 2), 2048)
        return pltpu.make_async_copy(wq_hbm.at[r, c], wqb.at[r, c], sem)

    def tail_copy(item, sem):
        if item[0] == "O":
            return row_copy(wo_hbm, wob, item[1], sem)
        src, dst = ((wg_hbm, wgb), (wu_hbm, wub), (wd_hbm, wdb))[item[1]]
        return row_copy(src, dst, item[2], sem)

    def a_copy(it, u):
        n = it - NQ
        if n < 0:
            return wq_copy(_QA[it * NU + u], sa(it))
        if n < NK:
            return k_copy(n, u)
        return tail_copy(_LATE_A[(n - NK) * NU + u], sa(it))

    def b_copy(it, u):
        n = it - NQ
        if n < 0:
            return wq_copy(_QB[it * NU + u], sb(it))
        if n < VOFF:
            return row_copy(wo_hbm, wob, u * VOFF + n, sb(it))
        if n < VOFF + NK:
            return v_copy(n - VOFF, u)
        item = _LATE_B[(n - VOFF - NK) * NU + u]
        if item[0] == "O" and item[1] >= 124:
            return row_copy(wo_hbm, wob, item[1], sem_x.at[3 + item[1] - 124])
        return tail_copy(item, sb(it))

    def issue(it):
        n = it - NQ
        for u in range(NU):
            if n < NA_END:
                a_copy(it, u).start(priority=0)
            if n < NB_END:
                b_copy(it, u).start(priority=1)

    def wait_tiles(ring, slot, sem):
        region = ring.at[pl.ds(slot, 2)]
        pltpu.make_async_copy(region, region, sem).wait()

    x_copy = pltpu.make_async_copy(x_hbm, xb, sem_x.at[0])
    wr_copy = pltpu.make_async_copy(wr_hbm, wrb, sem_x.at[1])
    x_copy.start()
    wr_copy.start()
    for it in range(DM):
        issue(it)

    x_copy.wait()
    x = xb[...].astype(F32)
    xc = x - jnp.mean(x, axis=-1, keepdims=True)
    xn = xc / jnp.sqrt(jnp.mean(xc * xc, axis=-1, keepdims=True) + 1e-5)
    xn_row = xn.astype(BF16)
    xn_lhs = jnp.broadcast_to(xn_row, (8, D))
    wr_copy.wait()
    r = jnp.sum(xn_row.astype(F32) * wrb[...].astype(F32).reshape(1, D), axis=-1, keepdims=True)
    r_gate = jax.nn.sigmoid(r)
    rows = lax.broadcasted_iota(jnp.int32, (8, 128), 0)

    q = None
    landed, slabs = set(), set()
    for it in range(NQ):
        issue(it + DM)
        for u in range(NU):
            a_copy(it, u).wait()
            b_copy(it, u).wait()
        landed.update(_QA[it * NU:(it + 1) * NU] + _QB[it * NU:(it + 1) * NU])
        for s in range(D // 128):
            if s not in slabs and all(32 * s + j in landed for j in range(32)):
                slabs.add(s)
                t = jnp.dot(xn_lhs[:, s * 128:(s + 1) * 128], wqb[pl.ds(s * 128, 128), :],
                            preferred_element_type=F32)
                q = t if q is None else q + t
    for h in range(H):
        q_scr[h] = q[:, h * DH:(h + 1) * DH]

    def score_tiles(n, s_idx, m, sc):
        sc = list(sc)
        base = k_slot(n)
        for k in range(NHS):
            qv = q_scr[NHS * s_idx + k].astype(BF16)
            for half in range(2):
                t = lax.dot_general(qv, kr[base + half, k], NT, preferred_element_type=F32)
                i = 4 * k + 2 * half
                sc[i] = jnp.where(rows == m, t, sc[i])
                sc[i + 1] = jnp.where(rows == m - 8, t, sc[i + 1])
        return sc

    def weighted_tiles(j, m, acc):
        acc = list(acc)
        base = v_slot(j)
        for k in range(NHS):
            for half in range(2):
                t = jnp.dot(p_scr[k, pl.ds(16 * half, 16), :], vr[base + half, k],
                            preferred_element_type=F32)
                if isinstance(m, int):
                    part = t[0:8] if m < 8 else t[8:16]
                    acc[k] = acc[k] + jnp.where(rows == m % 8, part, 0.0)
                else:
                    acc[k] = acc[k] + (jnp.where(rows == m, t[0:8], 0.0)
                                       + jnp.where(rows == m - 8, t[8:16], 0.0))
        return acc

    def softmax_set(sc):
        inv = []
        for k in range(NHS):
            c = jnp.concatenate(sc[4 * k:4 * k + 4], axis=0)
            p = jnp.exp2((c - jnp.max(c, axis=(0, 1), keepdims=True)) * score_scale)
            p_scr[k] = p.astype(BF16)
            inv.append(1.0 / jnp.sum(p, axis=(0, 1), keepdims=True))
        return tuple(inv)

    def normalize(acc, inv):
        return [jnp.broadcast_to(jnp.sum(acc[k], axis=0, keepdims=True) * inv[k], (8, DH)).astype(BF16)
                for k in range(NHS)]

    def out_proj(o_head, h):
        return jnp.dot(o_head, wob[pl.ds(aligned(h * DH, DH), DH), :], preferred_element_type=F32)

    zero_scores = (jnp.zeros((8, 128), F32),) * (4 * NHS)
    zero_acc = (jnp.zeros((8, 128), F32),) * NHS

    def first_set_step(m, sc):
        n2 = m + DM
        for u in range(NU):
            k_copy(n2, u).start(priority=0)

            @pl.when(n2 < VOFF)
            def _():
                row_copy(wo_hbm, wob, u * VOFF + n2, sb(NQ + n2)).start(priority=1)

            @pl.when(n2 >= VOFF)
            def _():
                v_copy(n2 - VOFF, u).start(priority=1)

        wait_tiles(kr, k_slot(m), sa(NQ + m))

        @pl.when(m < VOFF)
        def _():
            for u in range(NU):
                row_copy(wo_hbm, wob, u * VOFF + m, sb(NQ + m)).wait()

        @pl.when(m >= VOFF)
        def _():
            wait_tiles(vr, v_slot(m - VOFF), sb(NQ + m))

        return tuple(score_tiles(m, 0, m, sc))

    inv = softmax_set(list(lax.fori_loop(0, NM, first_set_step, zero_scores)))

    def run_set(s_idx):
        def step(m, carry):
            n = s_idx * NM + m
            n2 = n + DM
            for u in range(NU):
                @pl.when(n2 < NK)
                def _():
                    k_copy(n2, u).start(priority=0)

                @pl.when(n2 >= NK)
                def _():
                    mat, unit = _late_a_lookahead(n2 - NK, u)
                    tail_copy(("F", mat, unit), sa(NQ + n2)).start(priority=0)

                v_copy(n2 - VOFF, u).start(priority=1)
            wait_tiles(kr, k_slot(n), sa(NQ + n))
            wait_tiles(vr, v_slot(n - VOFF), sb(NQ + n))
            sc = score_tiles(n, s_idx, m, carry[0])
            acc = weighted_tiles(n - NM, m, carry[1])
            return tuple(sc), tuple(acc)
        return lax.fori_loop(0, NM, step, (zero_scores, zero_acc))

    def set_step(s_idx, carry):
        s_acc, inv_prev = carry
        sc, acc = run_set(s_idx)
        o_set = normalize(acc, inv_prev)
        for k in range(NHS):
            s_acc = s_acc + out_proj(o_set[k], NHS * (s_idx - 1) + k)
        return s_acc, softmax_set(list(sc))

    s_acc, inv = lax.fori_loop(1, NSET - 1, set_step, (jnp.zeros((8, D), F32), inv))
    sc, acc = run_set(NSET - 1)
    pending = [(o, NHS * (NSET - 2) + k) for k, o in enumerate(normalize(acc, inv))]
    inv = softmax_set(list(sc))

    extra_copy = tail_copy(_EXTRA, sem_x.at[2])
    extra_copy.start(priority=0)
    acc = list(zero_acc)
    v_next, a_next = NK - NM, NK
    have, act, y, gate, o_last = set(), {}, None, None, None
    for n in range(NK, NB_END):
        last = n == NB_END - 1
        issue(NQ + n + DM)
        while a_next < NA_END and (a_next <= n + SKEW or last):
            for u in range(NU):
                a_copy(NQ + a_next, u).wait()
            have.update(_LATE_A[(a_next - NK) * NU:(a_next - NK + 1) * NU])
            a_next += 1
        if n == NK:
            extra_copy.wait()
            have.add(_EXTRA)
        if n < VOFF + NK:
            wait_tiles(vr, v_slot(n - VOFF), sb(NQ + n))
        else:
            for u in range(NU // 2 if last else NU):
                b_copy(NQ + n, u).wait()
                have.add(_LATE_B[(n - VOFF - NK) * NU + u])

        budget = NM if n == VOFF + NK - 1 else 2
        while v_next <= min(n - VOFF, NK - 1) and budget > 0:
            acc = weighted_tiles(v_next, v_next % NM, acc)
            v_next, budget = v_next + 1, budget - 1
            if v_next == NK:
                o_set = normalize(acc, inv)
                pending += [(o_set[k], H - NHS + k) for k in range(NHS - 1)]
                o_last = o_set[NHS - 1]

        for c in range(11):
            units = range(4 * c, min(4 * c + 4, NFU))
            chunk = pl.ds(128 * c, FU * len(units))
            if c not in act and all(("F", m, i) in have for m in (0, 1) for i in units):
                g = lax.dot_general(xn_lhs, wgb[chunk, :], NT, preferred_element_type=F32)
                up = lax.dot_general(xn_lhs, wub[chunk, :], NT, preferred_element_type=F32)
                act[c] = ((g * jax.nn.sigmoid(g)) * up).astype(BF16)
            if act.get(c) is not None and all(("F", 2, i) in have for i in units):
                t = jnp.dot(act[c], wdb[chunk, :], preferred_element_type=F32)
                y = t if y is None else y + t
                act[c] = None
        if gate is None and len(act) == 11 and all(a is None for a in act.values()):
            routed = xn + (xn * 0.0 + y * r_gate)
            gate = routed * jax.nn.sigmoid(routed)

        for o_head, h in list(pending):
            if all(("O", w) in have for w in range(4 * h, 4 * h + 4)):
                s_acc = s_acc + out_proj(o_head, h)
                pending.remove((o_head, h))
    assert v_next == NK and a_next == NA_END and gate is not None and not pending

    o_col = jnp.transpose(jnp.broadcast_to(o_last.astype(F32)[0:1], (DH, DH)))
    part = None
    for j in range(4):
        row_copy(wo_hbm, wob, 124 + j, sem_x.at[3 + j]).wait()
        prod = wob[pl.ds((124 + j) * FU, FU), :].astype(F32) * jnp.concatenate(
            [o_col[j * FU:(j + 1) * FU]] * (D // 128), axis=1)
        for i in range(FU // 8):
            blk = prod[8 * i:8 * i + 8]
            part = blk if part is None else part + blk
    s = s_acc[0:1] + jnp.sum(part, axis=0, keepdims=True)

    o_ref[...] = (x + s * gate[0:1]).astype(o_ref.dtype)


@jax.jit
def pallas_recurrent_scan__sliding_block_cached__moe_arch_mod__decode_kernel(
    A_x: jax.Array,
    A_k_cache: jax.Array,
    A_v_cache: jax.Array,
    A_wq: jax.Array,
    A_wo: jax.Array,
    B_x: jax.Array,
    B_w_r: jax.Array,
    B_w_gate: jax.Array,
    B_w_up: jax.Array,
    B_w_down: jax.Array,
):
    del B_x
    assert A_x.shape == (1, 1, D) and A_k_cache.shape[:2] == (1, H) and A_k_cache.shape[3] == DH
    assert min(4096, max(256, A_k_cache.shape[2] // 4)) == W and A_k_cache.shape[2] % 128 == 0
    in_hbm = pl.BlockSpec(memory_space=pltpu.HBM)
    out = pl.pallas_call(
        _decode_kernel,
        out_shape=jax.ShapeDtypeStruct((1, D), A_x.dtype),
        in_specs=[in_hbm] * 9,
        out_specs=pl.BlockSpec(memory_space=pltpu.VMEM),
        scratch_shapes=[
            pltpu.VMEM((1, D), BF16),
            pltpu.VMEM((D,), BF16),
            pltpu.VMEM((D, H * DH), BF16),
            pltpu.VMEM((RS * 2, NHS, 128, DH), BF16),
            pltpu.VMEM((RV * 2, NHS, 128, DH), BF16),
            pltpu.VMEM((H * DH, D), BF16),
            pltpu.VMEM((FF, D), BF16),
            pltpu.VMEM((FF, D), BF16),
            pltpu.VMEM((FF, D), BF16),
            pltpu.VMEM((H, 8, DH), F32),
            pltpu.VMEM((NHS, 32, DH), BF16),
            pltpu.SemaphoreType.DMA((RS,)),
            pltpu.SemaphoreType.DMA((RS,)),
            pltpu.SemaphoreType.DMA((7,)),
        ],
        compiler_params=pltpu.CompilerParams(
            vmem_limit_bytes=48 * 1024 * 1024,
            disable_semaphore_checks=True,
        ),
        name="recurrent_scan_decode",
    )(
        A_x.reshape(1, D), A_k_cache, A_v_cache, A_wq, A_wo, B_w_r,
        B_w_gate.T, B_w_up.T, B_w_down,
    )
    return out.reshape(1, 1, D)
```
